```python
import os as _os
_os.environ.setdefault("JAX_PLATFORMS", "cpu")
import jax
import jax.numpy as jnp

def _softmax(x, axis=-1):
    return jax.nn.softmax(x, axis=axis)
def _gelu(x):
    return jax.nn.gelu(x, approximate=True)
def _silu(x):
    return jax.nn.silu(x)
def _sigmoid(x):
    return jax.nn.sigmoid(x)
def _layernorm(x, axis=-1, eps=1e-5):
    m = jnp.mean(x, axis=axis, keepdims=True)
    v = jnp.var(x, axis=axis, keepdims=True)
    return (x - m) / jnp.sqrt(v + eps)
def _scatter_add(tgt, idx, src, axis=0):
    return tgt.at[idx].add(src)
def _segment_sum(src, seg, n):
    return jax.ops.segment_sum(src, seg, n)
class _Rng:
    def __init__(self, key):
        self._k = key
    def _next(self):
        self._k, sub = jax.random.split(self._k)
        return sub
    def normal(self, shape):
        return jax.random.normal(self._next(), shape, dtype=jnp.bfloat16)
    def randint(self, lo, hi, shape):
        return jax.random.randint(self._next(), shape, lo, hi, dtype=jnp.int32)
    def uniform(self, shape, lo=0.0, hi=1.0):
        return jax.random.uniform(self._next(), shape, jnp.bfloat16, lo, hi)
    def permutation(self, n):
        return jax.random.permutation(self._next(), n)


kernel_name = 'sequential_preLN__mha_block__swiglu_ffn__prompt'

def setup_inputs():
    _rng = _Rng(jax.random.key(int.from_bytes(__import__("os").urandom(4), "little")))
    _w = (lambda a: (lambda t: t.astype(jnp.bfloat16) if jnp.issubdtype(t.dtype, jnp.floating) else t)(jnp.asarray(a)))
    def _A_setup():
        B, S, D, H = 1, 2048, 640, 32
        return {
            "x": _w((lambda *s: _rng.normal(s) * 0.05)(B, S, D)),
            "wqkv": _w((lambda *s: _rng.normal(s) * 0.05)(D, 3 * D)),
            "wo": _w((lambda *s: _rng.normal(s) * 0.05)(D, D)),
        }
    _A_in = _A_setup()

    def _B_setup():
        B, S, D, F = 1, 2048, 640, 1728
        return {
            "x": _w((lambda *s: _rng.normal(s) * 0.05)(B, S, D)),
            "w_gate": _w((lambda *s: _rng.normal(s) * 0.05)(D, F)),
            "w_up": _w((lambda *s: _rng.normal(s) * 0.05)(D, F)),
            "w_down": _w((lambda *s: _rng.normal(s) * 0.05)(F, D)),
        }
    _B_in = _B_setup()

    return {
        "A_x": _A_in["x"],
        "A_wqkv": _A_in["wqkv"],
        "A_wo": _A_in["wo"],
        "B_x": _B_in["x"],
        "B_w_gate": _B_in["w_gate"],
        "B_w_up": _B_in["w_up"],
        "B_w_down": _B_in["w_down"],
    }

def reference(A_x, A_wqkv, A_wo, B_x, B_w_gate, B_w_up, B_w_down):
    def _A_ref(x, wqkv, wo):
        B, S, D = x.shape
        H = 32
        Dh = D // H
        qkv = (lambda x, *d: x.transpose(*d))((x @ wqkv).reshape(B, S, 3, H, Dh), 2, 0, 3, 1, 4)
        q, k, v = qkv[0], qkv[1], qkv[2]
        scores = jnp.einsum("bhqd,bhkd->bhqk", q, k) * (Dh ** -0.5)
        p = _softmax(scores, axis=-1)
        o = jnp.einsum("bhqk,bhkd->bhqd", p, v)
        return (lambda x, *d: x.transpose(*d))(o, 0, 2, 1, 3).reshape(B, S, D) @ wo

    def _B_ref(x, w_gate, w_up, w_down):
        g = _silu(x @ w_gate)
        u = x @ w_up
        return (g * u) @ w_down

    x = A_x
    h = x + _A_ref(_layernorm(x, axis=-1), A_wqkv, A_wo)
    h2 = h + _B_ref(_layernorm(h, axis=-1), B_w_gate, B_w_up, B_w_down)
    return h2
```

```python
import functools
import math

import jax
import jax.numpy as jnp
from jax import lax
import jax.experimental.pallas as pl
import jax.experimental.pallas.tpu as pltpu

S = 2048
D = 640
H = 32
DH = 20
F = 1728
EPS = 1e-5

HPG = 6
NG = 6
TQ = 512
NQ = S // TQ
CK = 128
NC = S // CK
NU = NQ * H
UPI = 2
LAG = 2
RB1 = 256
RB2 = 256
FCH = (384, 384, 384, 384, 192)

QSCALE = (DH ** -0.5) * math.log2(math.e)

_NT = (((1,), (1,)), ((), ()))


def _layernorm(x):
    mu = jnp.mean(x, axis=-1, keepdims=True)
    xc = x - mu
    var = jnp.mean(xc * xc, axis=-1, keepdims=True)
    return xc * lax.rsqrt(var + EPS)


def _kernel(x_hbm, wqkv_hbm, wo_hbm, wg_hbm, wu_hbm, wd_hbm, out_hbm,
            x_ref, wqkv_ref, wo_ref, wg_ref, wu_ref, wd_ref,
            q_ref, k_ref, vt_ref, s0_ref, s1_ref, ot_ref, y_ref,
            z_ref, in_sems, out_sems):
    cp_x = pltpu.make_async_copy(x_hbm.at[0], x_ref, in_sems.at[0])
    cp_wqkv = pltpu.make_async_copy(wqkv_hbm, wqkv_ref, in_sems.at[1])
    cp_wo = pltpu.make_async_copy(wo_hbm, wo_ref, in_sems.at[2])
    cp_wg = pltpu.make_async_copy(wg_hbm, wg_ref, in_sems.at[3])
    cp_wu = pltpu.make_async_copy(wu_hbm, wu_ref, in_sems.at[4])
    cp_wd = pltpu.make_async_copy(wd_hbm, wd_ref, in_sems.at[5])
    cp_x.start()
    cp_wqkv.start()
    cp_x.wait()
    cp_wqkv.wait()
    cp_wo.start()
    cp_wg.start()
    cp_wu.start()
    cp_wd.start()
    z_ref[0] = 0

    row8 = lax.broadcasted_iota(jnp.int32, (8, RB1), 0)
    ones_hi = jnp.where(row8 == 4, 1.0, 0.0).astype(jnp.float32)
    ones_lo = jnp.where(row8 == 0, 1.0, 0.0).astype(jnp.float32)

    def qkv_block(rb, carry):
        r0 = pl.multiple_of(rb * RB1, RB1)
        x = x_ref[pl.ds(r0, RB1), :].astype(jnp.float32)
        xn = _layernorm(x).astype(jnp.bfloat16)
        qkv = jnp.dot(xn, wqkv_ref[...], preferred_element_type=jnp.float32)
        for g in range(NG):
            a = g * HPG * DH
            q_ref[g, pl.ds(r0, RB1), :] = (qkv[:, a:a + 128] * QSCALE).astype(jnp.bfloat16)
            k_ref[g, pl.ds(r0, RB1), :] = qkv[:, D + a:D + a + 128].astype(jnp.bfloat16)
        vt = qkv[:, 2 * D:3 * D].T
        for t in range(H // 2):
            b = 40 * t
            mid = vt[b + 16:b + 24]
            vt_ref[2 * t, rb, 0:16, :] = vt[b:b + 16]
            vt_ref[2 * t, rb, 16:24, :] = jnp.where(row8 < 4, mid, ones_hi)
            vt_ref[2 * t + 1, rb, 0:8, :] = jnp.where(row8 >= 4, mid, ones_lo)
            vt_ref[2 * t + 1, rb, 8:24, :] = vt[b + 24:b + 40]
        return carry

    lax.fori_loop(0, S // RB1, qkv_block, 0)

    lane = lax.broadcasted_iota(jnp.int32, (TQ, 128), 1)
    row8q = lax.broadcasted_iota(jnp.int32, (8, TQ), 0)

    def make_qm(u):
        qb = u // H
        h = u % H
        g = h // HPG
        j = h % HPG
        q = q_ref[g, pl.ds(pl.multiple_of(qb * TQ, TQ), TQ), :]
        mask = (lane >= j * DH) & (lane < j * DH + DH)
        return jnp.where(mask, q, jnp.zeros_like(q))

    def stage_a(u, qm, s_ref, c, mx):
        g = (u % H) // HPG
        k = k_ref[g, c * CK:(c + 1) * CK, :]
        s = lax.dot_general(k, qm, _NT, preferred_element_type=jnp.float32)
        s_ref[0, c * CK:(c + 1) * CK, :] = s
        cm = jnp.max(s.reshape(CK // 8, 8, TQ), axis=0)
        return cm if mx is None else jnp.maximum(mx, cm)

    def stage_b(u, z, s_ref, c, m, acc):
        h = u % H
        s = s_ref[z, c * CK:(c + 1) * CK, :]
        p = jnp.exp2(s.reshape(CK // 8, 8, TQ) - m[None]).reshape(CK, TQ).astype(jnp.bfloat16)
        rb, off = divmod(c * CK, RB1)
        vt = vt_ref[h, rb, :, off:off + CK]
        r = jnp.dot(vt, p, preferred_element_type=jnp.float32)
        return r if acc is None else acc + r

    def unit(u, z, mx_cur, s_cur, s_nxt):
        un = jnp.minimum(u + 1, NU - 1)
        qm = make_qm(un)
        m = jnp.broadcast_to(jnp.max(mx_cur, axis=0, keepdims=True), (8, TQ))
        mx = None
        acc = None
        for c in range(NC + LAG):
            if c < NC:
                mx = stage_a(un, qm, s_nxt, c, mx)
            if c >= LAG:
                acc = stage_b(u, z, s_cur, c - LAG, m, acc)
        return mx, acc

    qm0 = make_qm(0)
    mx0 = None
    for c in range(NC):
        mx0 = stage_a(0, qm0, s0_ref, c, mx0)

    def attn_iter(t, mx):
        z = z_ref[0]
        for i in range(0, UPI, 2):
            u = UPI * t + i
            mx, acc_e = unit(u, z, mx, s0_ref, s1_ref)
            mx, acc_o = unit(u + 1, z, mx, s1_ref, s0_ref)
            o_e = acc_e * (1.0 / acc_e[20:21])
            o_o = acc_o * (1.0 / acc_o[0:1])
            mid = jnp.where(row8q < 4, o_e[16:24], o_o[0:8])
            o = jnp.concatenate([o_e[0:16], mid, o_o[8:24]], axis=0)
            qb = u // H
            hp = (u % H) // 2
            ot_ref[qb, pl.ds(pl.multiple_of(hp * 40, 8), 40), :] = o
        return mx

    lax.fori_loop(0, NU // UPI, attn_iter, mx0)

    cp_wo.wait()
    cp_wg.wait()
    cp_wu.wait()
    cp_wd.wait()

    def out_copy(rb):
        r0 = pl.multiple_of(rb * RB2, RB2)
        return pltpu.make_async_copy(y_ref.at[pl.ds(r0, RB2), :],
                                     out_hbm.at[0, pl.ds(r0, RB2), :],
                                     out_sems.at[rb])

    def ffn_qblock(qb, carry):
        for sb in range(TQ // RB2):
            rb = qb * (TQ // RB2) + sb
            r0 = pl.multiple_of(rb * RB2, RB2)
            o = ot_ref[qb, :, sb * RB2:(sb + 1) * RB2].T.astype(jnp.bfloat16)
            hres = x_ref[pl.ds(r0, RB2), :].astype(jnp.float32) + jnp.dot(
                o, wo_ref[...], preferred_element_type=jnp.float32)
            hn = _layernorm(hres).astype(jnp.bfloat16)
            acc = hres
            f0 = 0
            for fw in FCH:
                g = jnp.dot(hn, wg_ref[:, f0:f0 + fw], preferred_element_type=jnp.float32)
                u = jnp.dot(hn, wu_ref[:, f0:f0 + fw], preferred_element_type=jnp.float32)
                a = (g * jax.nn.sigmoid(g) * u).astype(jnp.bfloat16)
                acc = acc + jnp.dot(a, wd_ref[f0:f0 + fw, :], preferred_element_type=jnp.float32)
                f0 += fw
            y_ref[pl.ds(r0, RB2), :] = acc.astype(y_ref.dtype)
            out_copy(rb).start()
        return carry

    lax.fori_loop(0, NQ, ffn_qblock, 0)
    for rb in range(S // RB2):
        out_copy(rb).wait()


@jax.jit
def pallas_sequential_preLN__mha_block__swiglu_ffn__prompt_kernel(
    A_x: jax.Array,
    A_wqkv: jax.Array,
    A_wo: jax.Array,
    B_x: jax.Array,
    B_w_gate: jax.Array,
    B_w_up: jax.Array,
    B_w_down: jax.Array,
):
    del B_x
    bf16 = jnp.bfloat16
    f32 = jnp.float32
    any_spec = pl.BlockSpec(memory_space=pl.ANY)
    return pl.pallas_call(
        _kernel,
        out_shape=jax.ShapeDtypeStruct((1, S, D), bf16),
        in_specs=[any_spec] * 6,
        out_specs=any_spec,
        scratch_shapes=[
            pltpu.VMEM((S, D), bf16),
            pltpu.VMEM((D, 3 * D), bf16),
            pltpu.VMEM((D, D), bf16),
            pltpu.VMEM((D, F), bf16),
            pltpu.VMEM((D, F), bf16),
            pltpu.VMEM((F, D), bf16),
            pltpu.VMEM((NG, S, 128), bf16),
            pltpu.VMEM((NG, S, 128), bf16),
            pltpu.VMEM((H, S // RB1, 24, RB1), f32),
            pltpu.VMEM((1, S, TQ), f32),
            pltpu.VMEM((1, S, TQ), f32),
            pltpu.VMEM((NQ, D, TQ), f32),
            pltpu.VMEM((S, D), bf16),
            pltpu.SMEM((1,), jnp.int32),
            pltpu.SemaphoreType.DMA((6,)),
            pltpu.SemaphoreType.DMA((S // RB2,)),
        ],
        compiler_params=pltpu.CompilerParams(vmem_limit_bytes=100 * 1024 * 1024),
    )(A_x, A_wqkv, A_wo, B_w_gate, B_w_up, B_w_down)
```

```python
import math

import jax
import jax.numpy as jnp
from jax import lax
import jax.experimental.pallas as pl
import jax.experimental.pallas.tpu as pltpu

S = 2048
D = 640
H = 32
DH = 20
F = 1728
EPS = 1e-5

TQ = 512
NQ = S // TQ
CK = 128
NC = S // CK
LAG = 2
RB1 = 512
SB1 = 128
RB2 = 512
SB2 = 256
FM = 1664
FCH = (384, 384, 384, 512)

N0 = 19
N2 = 5
N2A = 3
QA = 1
NR = 19
NPM = 4
NSTEP = 2 * NQ * NC
BIG = frozenset(int(round(k * NC / N2)) for k in range(N2))
BIGA = frozenset(int(round(k * NC / N2A)) for k in range(N2A))

SAFE_BOUND = 64.0
V_LO = 2.0 ** -30
V_HI = 2.0 ** 40

QSCALE = (DH ** -0.5) * math.log2(math.e)

_NT = (((1,), (1,)), ((), ()))
bf16 = jnp.bfloat16
f32 = jnp.float32
u32 = jnp.uint32

STEPS = [(i, qb, c) for i in range(2) for qb in range(NQ) for c in range(NC)]


def _vr(n):
    i, qb, c = STEPS[n]
    if n < N0:
        return 0
    if i == 1 and c in BIG:
        return 32
    if i == 0 and qb >= QA and c in BIGA:
        return 32
    return 16


def _nblk(i, c):
    return max(_vr(n) for n in range(NSTEP) if STEPS[n][0] == i and STEPS[n][2] == c) // 16


KB_IDX = {}
for _i in range(2):
    for _c in range(NC):
        for _b in range(_nblk(_i, _c)):
            KB_IDX[(_i, _c, _b)] = len(KB_IDX)
PV_OFF = [0]
for _n in range(NSTEP):
    PV_OFF.append(PV_OFF[-1] + _vr(_n))


def _layernorm(x):
    mu = jnp.mean(x, axis=-1, keepdims=True)
    xc = x - mu
    var = jnp.mean(xc * xc, axis=-1, keepdims=True)
    return xc * lax.rsqrt(var + EPS)


def _pack(x):
    return pltpu.bitcast(x.astype(bf16), u32)


def _kernel(x_hbm, wqkv_hbm, wo_hbm, wgt_hbm, wut_hbm, wd_hbm, out_hbm,
            x_ref, wqkv_ref, wo_ref, wgu_ref, wd_ref,
            k_ref, qtb_ref, qtf_ref, vt_ref, kb_ref, pv_ref, pm0_ref, pm1_ref, pm2_ref, pm3_ref, px_ref,
            s0_ref, s1_ref, ot_ref, y_ref, xn_ref, h_ref, hn_ref,
            z_ref, in_sems, out_sems):
    nxb = S // RB1
    cp_x = [pltpu.make_async_copy(x_hbm.at[0, pl.ds(b * RB1, RB1), :],
                                  x_ref.at[pl.ds(b * RB1, RB1), :], in_sems.at[b])
            for b in range(nxb)]
    cp_w = [pltpu.make_async_copy(wqkv_hbm.at[:, pl.ds(p * D, D)], wqkv_ref.at[:, pl.ds(p * D, D)],
                                  in_sems.at[nxb + p]) for p in range(3)]
    l0 = nxb + 3
    ft = F - FM
    late = [
        pltpu.make_async_copy(wo_hbm, wo_ref, in_sems.at[l0]),
        pltpu.make_async_copy(wgt_hbm.at[pl.ds(0, FM), :], wgu_ref.at[pl.ds(0, FM), :], in_sems.at[l0 + 1]),
        pltpu.make_async_copy(wut_hbm.at[pl.ds(0, FM), :], wgu_ref.at[pl.ds(FM, FM), :], in_sems.at[l0 + 2]),
        pltpu.make_async_copy(wgt_hbm.at[pl.ds(FM, ft), :], wgu_ref.at[pl.ds(2 * FM, ft), :],
                              in_sems.at[l0 + 3]),
        pltpu.make_async_copy(wut_hbm.at[pl.ds(FM, ft), :], wgu_ref.at[pl.ds(2 * FM + ft, ft), :],
                              in_sems.at[l0 + 4]),
        pltpu.make_async_copy(wd_hbm, wd_ref, in_sems.at[l0 + 5]),
    ]
    for cp in (cp_x[0], cp_w[2], cp_w[0], cp_w[1], cp_x[1], cp_x[2], cp_x[3]):
        cp.start()
    z_ref[0] = 0

    def ln1(rb, sb):
        rows = slice(rb * RB1 + sb * SB1, rb * RB1 + (sb + 1) * SB1)
        xn_ref[rows, :] = _layernorm(x_ref[rows, :].astype(f32)).astype(bf16)

    row8 = lax.broadcasted_iota(jnp.int32, (8, SB1), 0)
    ones_hi = jnp.where(row8 == 4, 1.0, 0.0).astype(f32)
    ones_lo = jnp.where(row8 == 0, 1.0, 0.0).astype(f32)
    zero8 = jnp.zeros((8, SB1), f32)

    def proj(rb, sb, p):
        rows = slice(rb * RB1 + sb * SB1, rb * RB1 + (sb + 1) * SB1)
        return jnp.dot(xn_ref[rows, :], wqkv_ref[:, p * D:(p + 1) * D], preferred_element_type=f32)

    def norm2_max(xt, cur):
        sq = xt * xt
        for t in range(H // 2):
            b = 40 * t
            amid = sq[b + 16:b + 24]
            ne = sq[b:b + 8] + sq[b + 8:b + 16] + jnp.where(row8 < 4, amid, zero8)
            no = sq[b + 24:b + 32] + sq[b + 32:b + 40] + jnp.where(row8 >= 4, amid, zero8)
            cur = jnp.maximum(cur, jnp.maximum(jnp.sum(ne, axis=0, keepdims=True),
                                               jnp.sum(no, axis=0, keepdims=True)))
        return cur

    def do_v(rb, sb, vmax):
        cs = slice(sb * SB1, (sb + 1) * SB1)
        v = proj(rb, sb, 2)
        vt = v.T
        for t in range(H // 2):
            b = 40 * t
            mid = vt[b + 16:b + 24]
            vt_ref[2 * t, rb, 0:16, cs] = vt[b:b + 16]
            vt_ref[2 * t, rb, 16:24, cs] = jnp.where(row8 < 4, mid, ones_hi)
            vt_ref[2 * t + 1, rb, 0:8, cs] = jnp.where(row8 >= 4, mid, ones_lo)
            vt_ref[2 * t + 1, rb, 8:24, cs] = vt[b + 24:b + 40]
        return jnp.maximum(vmax, jnp.max(jnp.abs(v).reshape(SB1 // 8, 8, D), axis=0))

    def do_q(rb, sb, qmax):
        cs = slice(sb * SB1, (sb + 1) * SB1)
        qt = (proj(rb, sb, 0) * QSCALE).T
        for t in range(H // 2):
            b = 40 * t
            qtf_ref[t, rb, :, cs] = qt[b:b + 40]
            qmid = qt[b + 16:b + 24]
            qe = jnp.concatenate([qt[b:b + 16], jnp.where(row8 < 4, qmid, zero8), zero8], axis=0)
            qo = jnp.concatenate([jnp.where(row8 >= 4, qmid, zero8), qt[b + 24:b + 40], zero8], axis=0)
            qtb_ref[t, rb, 0:16, cs] = _pack(qe)
            qtb_ref[t, rb, 16:32, cs] = _pack(qo)
        return norm2_max(qt, qmax)

    def do_k(rb, sb, kmax):
        k = proj(rb, sb, 1)
        kp = _pack(k)
        rp = rb * (RB1 // 2) + sb * (SB1 // 2)
        for t in range(H // 2):
            off = 2 * DH * t
            tl, lo = divmod(off, 128)
            if lo + 2 * DH <= 128:
                win = kp[:, tl * 128:(tl + 1) * 128]
                if lo:
                    win = pltpu.roll(win, 128 - lo, 1)
            else:
                win = kp[:, off:off + 128]
            k_ref[t, rp:rp + SB1 // 2, :] = win
        return norm2_max(k.T, kmax)

    nsb = RB1 // SB1
    qmax = jnp.zeros((1, SB1), f32)
    kmax = jnp.zeros((1, SB1), f32)
    vmax = jnp.zeros((8, D), f32)

    cp_x[0].wait()
    for sb in range(nsb):
        ln1(0, sb)
    cp_w[2].wait()
    for sb in range(nsb):
        vmax = do_v(0, sb, vmax)
    cp_w[0].wait()
    for sb in range(nsb):
        qmax = do_q(0, sb, qmax)
    cp_w[1].wait()
    cp_x[1].wait()
    cp_x[2].wait()
    for sb in range(nsb):
        kmax = do_k(0, sb, kmax)
        ln1(1, sb)
    for sb in range(nsb):
        kmax = do_k(1, sb, kmax)
        qmax = do_q(1, sb, qmax)
        vmax = do_v(1, sb, vmax)
        ln1(2, sb)

    cp_x[3].wait()
    for cp in late:
        cp.start()
    for rb in range(2, nxb):
        for sb in range(nsb):
            kmax = do_k(rb, sb, kmax)
            qmax = do_q(rb, sb, qmax)
            vmax = do_v(rb, sb, vmax)
            if rb + 1 < nxb:
                ln1(rb + 1, sb)

    zero_w = jnp.zeros((8, TQ), u32)

    def qk_mxu(t, i, qb, lo, hi):
        k = pltpu.bitcast(k_ref[t, lo // 2:hi // 2, :], bf16)
        if i == 0:
            qm = pltpu.bitcast(qtb_ref[t, qb, 0:16, :], bf16)
            return jnp.dot(k[:, :32], qm, preferred_element_type=f32)
        qm = pltpu.bitcast(jnp.concatenate([zero_w, qtb_ref[t, qb, 16:32, :]], axis=0), bf16)
        return jnp.dot(k[:, :48], qm, preferred_element_type=f32)

    def head_steps(t, n):
        i, qb, c = STEPS[n]
        px_ref[n] = jnp.exp2(qk_mxu(t, i, qb, c * CK, (c + 1) * CK))

    for n in range(LAG):
        head_steps(0, n)

    bound2 = jnp.max(qmax) * jnp.max(kmax) * 1.02
    vm = jnp.max(vmax)
    fast_ok = (bound2 <= SAFE_BOUND * SAFE_BOUND) & (vm >= V_LO) & (vm <= V_HI)

    row8q = lax.broadcasted_iota(jnp.int32, (8, TQ), 0)

    def pv(h, p, c, acc):
        rb, off = divmod(c * CK, RB1)
        vt = vt_ref[h, rb, :, off:off + CK]
        r = jnp.dot(vt, p, preferred_element_type=f32)
        return r if acc is None else acc + r

    def store_pair(t, qb, acc_e, acc_o):
        o_e = acc_e * (1.0 / acc_e[20:21])
        o_o = acc_o * (1.0 / acc_o[0:1])
        mid = jnp.where(row8q < 4, o_e[16:24], o_o[0:8])
        o = jnp.concatenate([o_e[0:16], mid, o_o[8:24]], axis=0)
        ot_ref[qb, pl.ds(pl.multiple_of(t * 40, 8), 40), :] = o

    def fast_attention():
        pms = (pm0_ref, pm1_ref, pm2_ref, pm3_ref)

        def gen(t, i):
            blocks = [key for key in KB_IDX if key[0] == i]
            kks = {}
            for key in blocks:
                r0 = (key[1] * CK + key[2] * 16) // 2
                kks[key] = k_ref[t, r0:r0 + 8, :]
            for d in range(DH):
                for key in blocks:
                    w = jnp.broadcast_to(kks[key][:, DH * i + d:DH * i + d + 1], (8, 128))
                    kb_ref[0, KB_IDX[key], d] = pltpu.bitcast(w, bf16).astype(f32)

        def qk_vpu(t, n, z):
            i, qb, c = STEPS[n]
            for b in range(_vr(n) // 16):
                accs = [None] * 4
                for d in range(DH):
                    kbc = kb_ref[z, KB_IDX[(i, c, b)], d].reshape(2, 8, 128)
                    for j in range(4):
                        qrow = jnp.broadcast_to(
                            qtf_ref[t, qb, i * DH + d:i * DH + d + 1, j * 128:(j + 1) * 128], (8, 128))
                        prod = kbc * qrow[None]
                        accs[j] = prod if accs[j] is None else accs[j] + prod
                sv = jnp.concatenate([a.reshape(16, 128) for a in accs], axis=1)
                r0 = PV_OFF[n] + b * 16
                pv_ref[0, r0:r0 + 16, :] = jnp.exp2(sv)

        def pair(t, carry):
            z = z_ref[0]
            hs = (2 * t, 2 * t + 1)
            gen(t, 0)
            gen(t, 1)
            accs = {}
            es = {}

            def finish(n):
                i, qb, c = STEPS[n]
                if n < LAG:
                    e = px_ref[n]
                elif n < NR:
                    e = es.pop(n)
                else:
                    e = pms[n % NPM][z, 0:CK - _vr(n), :]
                if _vr(n):
                    e = jnp.concatenate([pv_ref[z, PV_OFF[n]:PV_OFF[n + 1], :], e], axis=0)
                accs[(i, qb)] = pv(hs[i], e.astype(bf16), c, accs.get((i, qb)))
                if c == NC - 1 and i == 1:
                    store_pair(t, qb, accs.pop((0, qb)), accs.pop((1, qb)))

            for n in range(LAG, NSTEP):
                i, qb, c = STEPS[n]
                qk_vpu(t, n, z)
                e = jnp.exp2(qk_mxu(t, i, qb, c * CK + _vr(n), (c + 1) * CK))
                if n < NR:
                    es[n] = e
                else:
                    pms[n % NPM][0, 0:CK - _vr(n), :] = e
                finish(n - LAG)
            tn = jnp.minimum(t + 1, H // 2 - 1)
            for n in range(LAG):
                head_steps(tn, n)
                finish(NSTEP - LAG + n)
            return carry

        lax.fori_loop(0, H // 2, pair, 0)

    def safe_attention():
        nu = NQ * H

        def stage_a(u, par, s_ref, c, mx):
            s = qk_mxu((u % H) // 2, par, u // H, c * CK, (c + 1) * CK)
            s_ref[0, c * CK:(c + 1) * CK, :] = s
            cm = jnp.max(s.reshape(CK // 8, 8, TQ), axis=0)
            return cm if mx is None else jnp.maximum(mx, cm)

        def stage_b(u, z, s_ref, c, m, acc):
            s = s_ref[z, c * CK:(c + 1) * CK, :]
            p = jnp.exp2(s.reshape(CK // 8, 8, TQ) - m[None]).reshape(CK, TQ).astype(bf16)
            return pv(u % H, p, c, acc)

        def unit(u, par, z, mx_cur, s_cur, s_nxt):
            un = jnp.minimum(u + 1, nu - 1)
            m = jnp.broadcast_to(jnp.max(mx_cur, axis=0, keepdims=True), (8, TQ))
            mx = None
            acc = None
            for c in range(NC + LAG):
                if c < NC:
                    mx = stage_a(un, 1 - par, s_nxt, c, mx)
                if c >= LAG:
                    acc = stage_b(u, z, s_cur, c - LAG, m, acc)
            return mx, acc

        mx0 = None
        for c in range(NC):
            mx0 = stage_a(0, 0, s0_ref, c, mx0)

        def attn_iter(it, mx):
            z = z_ref[0]
            u = 2 * it
            mx, acc_e = unit(u, 0, z, mx, s0_ref, s1_ref)
            mx, acc_o = unit(u + 1, 1, z, mx, s1_ref, s0_ref)
            store_pair((u % H) // 2, u // H, acc_e, acc_o)
            return mx

        lax.fori_loop(0, nu // 2, attn_iter, mx0)

    pl.when(fast_ok)(fast_attention)
    pl.when(jnp.logical_not(fast_ok))(safe_attention)

    for cp in late:
        cp.wait()

    def out_copy(rb):
        r0 = pl.multiple_of(rb * SB2, SB2)
        return pltpu.make_async_copy(y_ref.at[pl.ds(r0, SB2), :],
                                     out_hbm.at[0, pl.ds(r0, SB2), :],
                                     out_sems.at[rb])

    def nt(a, w):
        return lax.dot_general(a, w, _NT, preferred_element_type=f32)

    for rb in range(S // SB2):
        qb, sb = divmod(rb, TQ // SB2)
        rows = slice(rb * SB2, (rb + 1) * SB2)
        o = ot_ref[qb, :, sb * SB2:(sb + 1) * SB2].T.astype(bf16)
        hres = x_ref[rows, :].astype(f32) + jnp.dot(o, wo_ref[...], preferred_element_type=f32)
        h_ref[rows, :] = hres
        hn_ref[rows, :] = _layernorm(hres).astype(bf16)

    def ffn_qblock(qb, carry):
        for sb in range(RB2 // SB2):
            rb = qb * (RB2 // SB2) + sb
            r0 = pl.multiple_of(rb * SB2, SB2)
            hn = hn_ref[pl.ds(r0, SB2), :]
            acc = h_ref[pl.ds(r0, SB2), :]
            gu = nt(hn, wgu_ref[2 * FM:2 * F, :])
            g = gu[:, 0:F - FM]
            u = gu[:, F - FM:2 * (F - FM)]
            a_prev = (g * jax.nn.sigmoid(g) * u).astype(bf16)
            w_prev = (FM, F)
            f0 = 0
            for fw in FCH:
                g = nt(hn, wgu_ref[f0:f0 + fw, :])
                u = nt(hn, wgu_ref[FM + f0:FM + f0 + fw, :])
                acc = acc + jnp.dot(a_prev, wd_ref[w_prev[0]:w_prev[1], :], preferred_element_type=f32)
                a_prev = (g * jax.nn.sigmoid(g) * u).astype(bf16)
                w_prev = (f0, f0 + fw)
                f0 += fw
            acc = acc + jnp.dot(a_prev, wd_ref[w_prev[0]:w_prev[1], :], preferred_element_type=f32)
            y_ref[pl.ds(r0, SB2), :] = acc.astype(y_ref.dtype)
            out_copy(rb).start()
        return carry

    lax.fori_loop(0, S // RB2, ffn_qblock, 0)
    for rb in range(S // SB2):
        out_copy(rb).wait()


@jax.jit
def pallas_sequential_preLN__mha_block__swiglu_ffn__prompt_kernel(
    A_x: jax.Array,
    A_wqkv: jax.Array,
    A_wo: jax.Array,
    B_x: jax.Array,
    B_w_gate: jax.Array,
    B_w_up: jax.Array,
    B_w_down: jax.Array,
):
    del B_x
    assert RB1 == TQ and RB2 == TQ and S // RB1 == 4 and LAG <= N0 <= NR
    hbm_spec = pl.BlockSpec(memory_space=pltpu.MemorySpace.HBM)
    return pl.pallas_call(
        _kernel,
        out_shape=jax.ShapeDtypeStruct((1, S, D), bf16),
        in_specs=[hbm_spec] * 6,
        out_specs=hbm_spec,
        scratch_shapes=[
            pltpu.VMEM((S, D), bf16),
            pltpu.VMEM((D, 3 * D), bf16),
            pltpu.VMEM((D, D), bf16),
            pltpu.VMEM((2 * F, D), bf16),
            pltpu.VMEM((F, D), bf16),
            pltpu.VMEM((H // 2, S // 2, 128), u32),
            pltpu.VMEM((H // 2, NQ, 32, TQ), u32),
            pltpu.VMEM((H // 2, NQ, 40, TQ), f32),
            pltpu.VMEM((H, NQ, 24, TQ), f32),
            pltpu.VMEM((1, len(KB_IDX), DH, 16, 128), f32),
            pltpu.VMEM((1, PV_OFF[-1], TQ), f32),
            pltpu.VMEM((1, CK, TQ), f32),
            pltpu.VMEM((1, CK, TQ), f32),
            pltpu.VMEM((1, CK, TQ), f32),
            pltpu.VMEM((1, CK, TQ), f32),
            pltpu.VMEM((LAG, CK, TQ), f32),
            pltpu.VMEM((1, S, TQ), f32),
            pltpu.VMEM((1, S, TQ), f32),
            pltpu.VMEM((NQ, D, TQ), f32),
            pltpu.VMEM((S, D), bf16),
            pltpu.VMEM((S, D), bf16),
            pltpu.VMEM((S, D), f32),
            pltpu.VMEM((S, D), bf16),
            pltpu.SMEM((1,), jnp.int32),
            pltpu.SemaphoreType.DMA((S // RB1 + 9,)),
            pltpu.SemaphoreType.DMA((S // SB2,)),
        ],
        compiler_params=pltpu.CompilerParams(vmem_limit_bytes=120 * 1024 * 1024),
    )(A_x, A_wqkv, A_wo, B_w_gate.T, B_w_up.T, B_w_down)
```
